```python
import os as _os
_os.environ.setdefault("JAX_PLATFORMS", "cpu")
import jax
import jax.numpy as jnp

def _softmax(x, axis=-1):
    return jax.nn.softmax(x, axis=axis)
def _gelu(x):
    return jax.nn.gelu(x, approximate=True)
def _silu(x):
    return jax.nn.silu(x)
def _sigmoid(x):
    return jax.nn.sigmoid(x)
def _layernorm(x, axis=-1, eps=1e-5):
    m = jnp.mean(x, axis=axis, keepdims=True)
    v = jnp.var(x, axis=axis, keepdims=True)
    return (x - m) / jnp.sqrt(v + eps)
def _scatter_add(tgt, idx, src, axis=0):
    return tgt.at[idx].add(src)
def _segment_sum(src, seg, n):
    return jax.ops.segment_sum(src, seg, n)
class _Rng:
    def __init__(self, key):
        self._k = key
    def _next(self):
        self._k, sub = jax.random.split(self._k)
        return sub
    def normal(self, shape):
        return jax.random.normal(self._next(), shape, dtype=jnp.bfloat16)
    def randint(self, lo, hi, shape):
        return jax.random.randint(self._next(), shape, lo, hi, dtype=jnp.int32)
    def uniform(self, shape, lo=0.0, hi=1.0):
        return jax.random.uniform(self._next(), shape, jnp.bfloat16, lo, hi)
    def permutation(self, n):
        return jax.random.permutation(self._next(), n)


kernel_name = 'concat_heads__gqa_block_cached__gqa_block_cached__near_ridge'

def setup_inputs():
    _rng = _Rng(jax.random.key(int.from_bytes(__import__("os").urandom(4), "little")))
    _w = (lambda a: (lambda t: t.astype(jnp.bfloat16) if jnp.issubdtype(t.dtype, jnp.floating) else t)(jnp.asarray(a)))
    def _A_setup():
        B, Sq, D = 16, 144, 448
        Hq, Hkv, Sk, Dh = 16, 8, 1024, 256
        assert Hq % Hkv == 0, (Hq, Hkv)
        return {
            "x": _w((lambda *s: _rng.normal(s) * 0.8)(B, Sq, D)),
            "k_cache": _w((lambda *s: _rng.normal(s) * 0.8)(B, Hkv, Sk, Dh)),
            "v_cache": _w((lambda *s: _rng.normal(s) * 0.05)(B, Hkv, Sk, Dh)),
            "wq": _w((lambda *s: _rng.normal(s) * 0.8)(D, Hq * Dh) * (D ** -0.5)),
            "wo": _w((lambda *s: _rng.normal(s) * 0.05)(Hq * Dh, D) * ((Hq * Dh) ** -0.5)),
        }
    _A_in = _A_setup()

    def _B_setup():
        B, Sq, D = 16, 144, 448
        Hq, Hkv, Sk, Dh = 16, 8, 1024, 256
        assert Hq % Hkv == 0, (Hq, Hkv)
        return {
            "x": _w((lambda *s: _rng.normal(s) * 0.8)(B, Sq, D)),
            "k_cache": _w((lambda *s: _rng.normal(s) * 0.8)(B, Hkv, Sk, Dh)),
            "v_cache": _w((lambda *s: _rng.normal(s) * 0.05)(B, Hkv, Sk, Dh)),
            "wq": _w((lambda *s: _rng.normal(s) * 0.8)(D, Hq * Dh) * (D ** -0.5)),
            "wo": _w((lambda *s: _rng.normal(s) * 0.05)(Hq * Dh, D) * ((Hq * Dh) ** -0.5)),
        }
    _B_in = _B_setup()

    return {
        "A_x": _A_in["x"],
        "A_k_cache": _A_in["k_cache"],
        "A_v_cache": _A_in["v_cache"],
        "A_wq": _A_in["wq"],
        "A_wo": _A_in["wo"],
        "B_x": _B_in["x"],
        "B_k_cache": _B_in["k_cache"],
        "B_v_cache": _B_in["v_cache"],
        "B_wq": _B_in["wq"],
        "B_wo": _B_in["wo"],
    }

def reference(A_x, A_k_cache, A_v_cache, A_wq, A_wo, B_x, B_k_cache, B_v_cache, B_wq, B_wo):
    def _A_ref(x, k_cache, v_cache, wq, wo):
        B, Sq, D = x.shape
        Hq, Dh = 16, 256
        Hkv = k_cache.shape[1]
        rep = Hq // Hkv
        q = (lambda x, *d: x.transpose(*d))((x @ wq).reshape(B, Sq, Hq, Dh), 0, 2, 1, 3)
        k = jnp.repeat(k_cache, rep, axis=1)
        v = jnp.repeat(v_cache, rep, axis=1)
        scores = jnp.einsum("bhqd,bhkd->bhqk", q, k) * (Dh ** -0.5)
        p = _softmax(scores, axis=-1)
        o = jnp.einsum("bhqk,bhkd->bhqd", p, v)
        return (lambda x, *d: x.transpose(*d))(o, 0, 2, 1, 3).reshape(B, Sq, Hq * Dh) @ wo

    def _B_ref(x, k_cache, v_cache, wq, wo):
        B, Sq, D = x.shape
        Hq, Dh = 16, 256
        Hkv = k_cache.shape[1]
        rep = Hq // Hkv
        q = (lambda x, *d: x.transpose(*d))((x @ wq).reshape(B, Sq, Hq, Dh), 0, 2, 1, 3)
        k = jnp.repeat(k_cache, rep, axis=1)
        v = jnp.repeat(v_cache, rep, axis=1)
        scores = jnp.einsum("bhqd,bhkd->bhqk", q, k) * (Dh ** -0.5)
        p = _softmax(scores, axis=-1)
        o = jnp.einsum("bhqk,bhkd->bhqd", p, v)
        return (lambda x, *d: x.transpose(*d))(o, 0, 2, 1, 3).reshape(B, Sq, Hq * Dh) @ wo

    a = _A_ref(A_x, A_k_cache, A_v_cache, A_wq, A_wo)
    b = _B_ref(B_x, B_k_cache, B_v_cache, B_wq, B_wo)
    return jnp.concatenate([a, b], axis=-1)
```

```python
import functools
import jax
import jax.numpy as jnp
import jax.experimental.pallas as pl
import jax.experimental.pallas.tpu as pltpu

LOG2E = 1.4426950408889634
NT = (((1,), (1,)), ((), ()))
BF16 = jnp.bfloat16
F32 = jnp.float32
NOBC = True
NC = 1
KS = 256
LAG = 1


@jax.jit
def pallas_concat_heads__gqa_block_cached__gqa_block_cached__near_ridge_kernel(
        A_x, A_k_cache, A_v_cache, A_wq, A_wo, B_x, B_k_cache, B_v_cache, B_wq, B_wo):
    A_k, A_v, B_k, B_v = A_k_cache, A_v_cache, B_k_cache, B_v_cache
    B, Sq, D = A_x.shape
    _, Hkv, Sk, Dh = A_k.shape
    HD = A_wq.shape[1]
    Hq = HD // Dh
    rep = Hq // Hkv
    scale = (Dh ** -0.5) * LOG2E
    W = rep * Dh
    M = B * Sq
    T = 128
    G = 8
    EX = Sq - T
    NQ = 4
    QW = HD // NQ
    U = 2 * Hkv
    CK = Sk // NC

    def kernel(ax, ak, av, awq, awo, bx, bk, bv, bwq, bwo, out, x_s, wq_s, q_s, wo_s, kv_s, out_s,
               sem_x, sem_wq, sem_wo, sem_kv, sem_out, *o_s):
        b = pl.program_id(0)
        j = b % G
        slot = b % 2
        kv_hbm = (ak, av, bk, bv)
        x_hbm = (ax, bx); wq_hbm = (awq, bwq); wo_hbm = (awo, bwo)

        def x_copy(blk):
            return pltpu.make_async_copy(x_hbm[blk], x_s.at[blk], sem_x.at[blk])

        def wq_copy(i):
            return pltpu.make_async_copy(wq_hbm[i // NQ].at[:, pl.ds((i % NQ) * QW, QW)], wq_s.at[i], sem_wq.at[i])

        def wo_copy(blk):
            return pltpu.make_async_copy(wo_hbm[blk], wo_s.at[blk], sem_wo.at[blk])

        def kv_copy(i, bb, s):
            return pltpu.make_async_copy(kv_hbm[i].at[bb], kv_s.at[s, i], sem_kv.at[s, i])

        def out_copy(s, t):
            return pltpu.make_async_copy(out_s.at[s], out.at[pl.ds(pl.multiple_of(t * T, T), T)], sem_out.at[s])

        @pl.when(b == 0)
        def _():
            x_copy(0).start()
            wq_copy(0).start()
            x_copy(0).wait()

            def q_iter(i, c):
                pltpu.make_async_copy(wq_hbm[0].at[:, pl.ds(0, QW)], wq_s.at[i], sem_wq.at[i]).wait()

                @pl.when(i == NQ)
                def _():
                    x_copy(1).wait()

                @pl.when(i == 0)
                def _():
                    for ii in range(1, 2 * NQ):
                        wq_copy(ii).start()
                    x_copy(1).start()

                @pl.when(i == 1)
                def _():
                    for blk in range(2):
                        wo_copy(blk).start()
                    for ii in range(4):
                        kv_copy(ii, 0, 0).start()

                @pl.when(i == 3)
                def _():
                    for ii in range(4):
                        kv_copy(ii, 1, 1).start()

                q = jnp.dot(x_s[i // NQ], wq_s[i], preferred_element_type=F32)
                q_s[i] = (q * scale).astype(BF16)
                return c

            jax.lax.fori_loop(0, 2 * NQ, q_iter, 0)
            for blk in range(2):
                wo_copy(blk).wait()

        for i in range(4):
            kv_copy(i, b, slot).wait()

        @pl.when(b >= 2)
        def _():
            out_copy(slot, 0).wait()

        row0 = pl.multiple_of(b * Sq, 16)
        orow = pl.multiple_of(j * EX, 16)

        def qk_part(u, lo, hi):
            blk, h = u % 2, u // 2
            qi, c0 = blk * NQ + (h * W) // QW, (h * W) % QW
            q = jnp.concatenate([q_s[qi, pl.ds(row0, Sq), c0 + r * Dh:c0 + (r + 1) * Dh] for r in range(rep)], axis=0)
            return jax.lax.dot_general(q, kv_s[slot, 2 * blk, h, lo:hi, :], NT, preferred_element_type=F32)

        def softmax(s):
            m = jnp.max(s, axis=-1, keepdims=True)
            p = jnp.exp2(s - m)
            l = jnp.sum(p, axis=-1, keepdims=True)
            return p.astype(BF16), l

        def pv(u, p, l):
            blk, h = u % 2, u // 2
            o = jnp.dot(p, kv_s[slot, 2 * blk + 1, h], preferred_element_type=F32)
            o = o * (1.0 / l)
            for r in range(rep):
                o_s[u][pl.ds(orow, Sq), r * Dh:(r + 1) * Dh] = o[r * Sq:(r + 1) * Sq].astype(BF16)

        def ot(u, r0):
            blk, h = u % 2, u // 2
            return jax.lax.dot_general(wo_s[blk, :, h * W:(h + 1) * W], o_s[u][r0:r0 + T, :], NT,
                                       preferred_element_type=F32)

        def emit(acc, s, t):
            out_s[s] = jnp.concatenate(acc, axis=0).T.astype(BF16)
            out_copy(s, t).start()

        P = {}
        acc = [None, None]

        def do_ot(u):
            r = ot(u, 0)
            o_s[u][0:T, :] = o_s[u][T:2 * T, :]
            acc[u % 2] = r if acc[u % 2] is None else acc[u % 2] + r

        for t in range(U + LAG):
            if t < U:
                sa = qk_part(t, 0, KS)
            if t >= LAG:
                do_ot(t - LAG)
            if t < U:
                sb = qk_part(t, KS, Sk)
                pv(t, *softmax(jnp.concatenate([sa, sb], axis=1)))

        @pl.when(b + 2 < B)
        def _():
            for i in range(4):
                kv_copy(i, b + 2, slot).start()

        emit(acc, slot, b + b // G)

        @pl.when(j == G - 1)
        def _():
            @pl.when(b > G)
            def _():
                out_copy(2, 0).wait()

            acc = [None, None]
            for u in range(U):
                r = ot(u, T)
                acc[u % 2] = r if acc[u % 2] is None else acc[u % 2] + r
            emit(acc, 2, b + b // G + 1)

        @pl.when(b == B - 1)
        def _():
            for s in range(3):
                out_copy(s, 0).wait()

    any_spec = pl.BlockSpec(memory_space=pl.ANY)
    out = pl.pallas_call(
        kernel,
        grid=(B,),
        in_specs=[any_spec] * 10,
        out_specs=any_spec,
        out_shape=jax.ShapeDtypeStruct((M, 2 * D), BF16),
        scratch_shapes=[
            pltpu.VMEM((2, M, D), BF16),
            pltpu.VMEM((2 * NQ, D, QW), BF16),
            pltpu.VMEM((2 * NQ, M, QW), BF16),
            pltpu.VMEM((2, D, HD), BF16),
            pltpu.VMEM((2, 4, Hkv, Sk, Dh), BF16),
            pltpu.VMEM((3, T, 2 * D), BF16),
            pltpu.SemaphoreType.DMA((2,)),
            pltpu.SemaphoreType.DMA((2 * NQ,)),
            pltpu.SemaphoreType.DMA((2,)),
            pltpu.SemaphoreType.DMA((2, 4)),
            pltpu.SemaphoreType.DMA((3,)),
        ] + [pltpu.VMEM((2 * T, W), BF16)] * U,
        compiler_params=pltpu.CompilerParams(
            dimension_semantics=("arbitrary",),
            vmem_limit_bytes=120 * 1024 * 1024,
            disable_bounds_checks=NOBC),
    )(A_x.reshape(M, D), A_k, A_v, A_wq, A_wo.T, B_x.reshape(M, D), B_k, B_v, B_wq, B_wo.T)
    return out.reshape(B, Sq, 2 * D)
```

```python
import jax
import jax.numpy as jnp
import jax.experimental.pallas as pl
import jax.experimental.pallas.tpu as pltpu

LOG2E = 1.4426950408889634
NT = (((1,), (1,)), ((), ()))
BF16 = jnp.bfloat16
F32 = jnp.float32
TL = "384"
DEPU = 1
OTPOS = 2


@jax.jit
def pallas_concat_heads__gqa_block_cached__gqa_block_cached__near_ridge_kernel(
        A_x, A_k_cache, A_v_cache, A_wq, A_wo, B_x, B_k_cache, B_v_cache, B_wq, B_wo):
    A_k, A_v, B_k, B_v = A_k_cache, A_v_cache, B_k_cache, B_v_cache
    B, Sq, D = A_x.shape
    _, Hkv, Sk, Dh = A_k.shape
    HD = A_wq.shape[1]
    Hq = HD // Dh
    rep = Hq // Hkv
    scale = (Dh ** -0.5) * LOG2E
    W = rep * Dh
    M = B * Sq
    T = 128
    G = 8
    EX = Sq - T
    NQ = 4
    QW = HD // NQ
    U = 2 * Hkv
    CK = 256
    NC = Sk // CK

    def kernel(ax, ak, av, awq, awo, bx, bk, bv, bwq, bwo, out, x_s, wq_s, q_s, wo_s, kv_s, out_s, acc_s,
               sem_x, sem_wq, sem_wo, sem_kv, sem_out, *o_s):
        b = pl.program_id(0)
        j = b % G
        slot = b % 2
        kv_hbm = (ak, av, bk, bv)
        x_hbm = (ax, bx); wq_hbm = (awq, bwq); wo_hbm = (awo, bwo)

        def x_copy(blk):
            return pltpu.make_async_copy(x_hbm[blk], x_s.at[blk], sem_x.at[blk])

        def wq_copy(i):
            return pltpu.make_async_copy(wq_hbm[i // NQ].at[:, pl.ds((i % NQ) * QW, QW)], wq_s.at[i], sem_wq.at[i])

        def wo_copy(blk):
            return pltpu.make_async_copy(wo_hbm[blk], wo_s.at[blk], sem_wo.at[blk])

        def kv_copy(i, bb, s):
            return pltpu.make_async_copy(kv_hbm[i].at[bb], kv_s.at[s, i], sem_kv.at[s, i])

        def out_copy(t):
            s = t % 2
            return pltpu.make_async_copy(out_s.at[s], out.at[pl.ds(pl.multiple_of(t * T, T), T)], sem_out.at[s])

        @pl.when(b == 0)
        def _():
            x_copy(0).start()
            wq_copy(0).start()
            acc_s[...] = jnp.zeros(acc_s.shape, F32)
            x_copy(0).wait()

            def q_iter(i, c):
                pltpu.make_async_copy(wq_hbm[0].at[:, pl.ds(0, QW)], wq_s.at[i], sem_wq.at[i]).wait()

                @pl.when(i == NQ)
                def _():
                    x_copy(1).wait()

                @pl.when(i == 0)
                def _():
                    for ii in range(1, 2 * NQ):
                        wq_copy(ii).start()
                    x_copy(1).start()

                @pl.when(i == 1)
                def _():
                    for blk in range(2):
                        wo_copy(blk).start()
                    for ii in range(4):
                        kv_copy(ii, 0, 0).start()

                @pl.when(i == 3)
                def _():
                    for ii in range(4):
                        kv_copy(ii, 1, 1).start()

                q = jnp.dot(x_s[i // NQ], wq_s[i], preferred_element_type=F32)
                q_s[i] = (q * scale).astype(BF16)
                return c

            jax.lax.fori_loop(0, 2 * NQ, q_iter, 0)
            for blk in range(2):
                wo_copy(blk).wait()

        for i in range(4):
            kv_copy(i, b, slot).wait()

        t_pend = jnp.maximum(b - 1 + b // G, 0)

        @pl.when(t_pend >= 2)
        def _():
            out_copy(t_pend).wait()

        zmask = b // B

        def tie(x):
            return pltpu.bitcast(pltpu.bitcast(x, jnp.int32) & zmask, F32)

        def stage(t):
            tt = acc_s[...].T
            out_s[t % 2] = tt.astype(BF16)
            z = tt[T - 8:T, 0:128]
            for i in range(1, 2 * D // 128):
                z = z + tt[T - 8:T, i * 128:(i + 1) * 128]
            return z

        zdep = stage(t_pend)

        @pl.when(b >= 1)
        def _():
            out_copy(t_pend).start()

        row0 = pl.multiple_of(b * Sq, 16)
        orow = pl.multiple_of(j * EX, 16)

        def qk_part(u, c):
            blk, h = u % 2, u // 2
            qi, c0 = blk * NQ + (h * W) // QW, (h * W) % QW
            q = jnp.concatenate([q_s[qi, pl.ds(row0, Sq), c0 + r * Dh:c0 + (r + 1) * Dh] for r in range(rep)], axis=0)
            return jax.lax.dot_general(q, kv_s[slot, 2 * blk, h, c * CK:(c + 1) * CK, :], NT, preferred_element_type=F32)

        def attend(u, s):
            blk, h = u % 2, u // 2
            m = jnp.max(s, axis=-1, keepdims=True)
            p = jnp.exp2(s - m)
            lp = p[:, 0:128]
            for i in range(1, Sk // 128):
                lp = lp + p[:, i * 128:(i + 1) * 128]
            o = None
            for c in range(NC):
                a = jnp.dot(p[:, c * CK:(c + 1) * CK].astype(BF16), kv_s[slot, 2 * blk + 1, h, c * CK:(c + 1) * CK, :],
                            preferred_element_type=F32)
                o = a if o is None else a + o
            lp = lp + tie(o[:, 0:128])
            if u == DEPU:
                lp = jnp.concatenate([lp[0:8] + tie(zdep), lp[8:]], axis=0)
            l = jnp.sum(lp, axis=-1, keepdims=True)
            o = o * (1.0 / l)
            for r in range(rep):
                o_s[u][pl.ds(orow, Sq), r * Dh:(r + 1) * Dh] = o[r * Sq:(r + 1) * Sq].astype(BF16)

        HB = D // 2

        def ot(u, r0, lo=0, hi=D):
            blk, h = u % 2, u // 2
            return jax.lax.dot_general(wo_s[blk, lo:hi, h * W:(h + 1) * W], o_s[u][r0:r0 + T, :], NT,
                                       preferred_element_type=F32)

        acc = [None, None]

        def shift(u):
            o_s[u][0:T, :] = o_s[u][T:2 * T, :]

        def do_ot(u):
            r = ot(u, 0)
            acc[u % 2] = r if acc[u % 2] is None else r + acc[u % 2]
            shift(u)

        splits = {U - 2 - i: int(x) for i, x in enumerate(TL.split(","))}
        lo_part = {}
        for t in range(U):
            ss = []
            for c in range(NC):
                if c == OTPOS and t >= 1:
                    u = t - 1
                    if u in splits:
                        n = D - splits[u]
                        lo_part[u] = ot(u, 0, 0, n) + acc[u % 2][0:n]
                    else:
                        do_ot(u)
                ss.append(qk_part(t, c))
            attend(t, jnp.concatenate(ss, axis=1))
        for u in sorted(splits):
            n = D - splits[u]
            hi = ot(u, 0, n, D) + acc[u % 2][n:D]
            acc[u % 2] = jnp.concatenate([lo_part[u], hi], axis=0)
            shift(u)
        do_ot(U - 1)
        acc_s[0:D, :] = acc[0]
        acc_s[D:2 * D, :] = acc[1]

        @pl.when(b + 2 < B)
        def _():
            for i in range(4):
                kv_copy(i, b + 2, slot).start()

        @pl.when(j == G - 1)
        def _():
            t1 = b + b // G
            out_copy(t1).wait()
            stage(t1)
            out_copy(t1).start()
            acc = [None, None]
            for u in range(U):
                r = ot(u, T)
                acc[u % 2] = r if acc[u % 2] is None else r + acc[u % 2]
            acc_s[0:D, :] = acc[0]
            acc_s[D:2 * D, :] = acc[1]

        @pl.when(b == B - 1)
        def _():
            t2 = M // T - 1
            out_copy(t2).wait()
            stage(t2)
            out_copy(t2).start()
            out_copy(t2 - 1).wait()
            out_copy(t2).wait()

    any_spec = pl.BlockSpec(memory_space=pl.ANY)
    out = pl.pallas_call(
        kernel,
        grid=(B,),
        in_specs=[any_spec] * 10,
        out_specs=any_spec,
        out_shape=jax.ShapeDtypeStruct((M, 2 * D), BF16),
        scratch_shapes=[
            pltpu.VMEM((2, M, D), BF16),
            pltpu.VMEM((2 * NQ, D, QW), BF16),
            pltpu.VMEM((2 * NQ, M, QW), BF16),
            pltpu.VMEM((2, D, HD), BF16),
            pltpu.VMEM((2, 4, Hkv, Sk, Dh), BF16),
            pltpu.VMEM((2, T, 2 * D), BF16),
            pltpu.VMEM((2 * D, T), F32),
            pltpu.SemaphoreType.DMA((2,)),
            pltpu.SemaphoreType.DMA((2 * NQ,)),
            pltpu.SemaphoreType.DMA((2,)),
            pltpu.SemaphoreType.DMA((2, 4)),
            pltpu.SemaphoreType.DMA((2,)),
        ] + [pltpu.VMEM((2 * T, W), BF16)] * U,
        compiler_params=pltpu.CompilerParams(
            dimension_semantics=("arbitrary",),
            vmem_limit_bytes=120 * 1024 * 1024,
            disable_bounds_checks=True),
    )(A_x.reshape(M, D), A_k, A_v, A_wq, A_wo.T, B_x.reshape(M, D), B_k, B_v, B_wq, B_wo.T)
    return out.reshape(B, Sq, 2 * D)
```

```python
import jax
import jax.numpy as jnp
from jax import lax
import jax.experimental.pallas as pl
import jax.experimental.pallas.tpu as pltpu

LOG2E = 1.4426950408889634
NT = (((1,), (1,)), ((), ()))
BF16 = jnp.bfloat16
F32 = jnp.float32
LANES = 128


@jax.jit
def pallas_concat_heads__gqa_block_cached__gqa_block_cached__near_ridge_kernel(
    A_x: jax.Array,
    A_k_cache: jax.Array,
    A_v_cache: jax.Array,
    A_wq: jax.Array,
    A_wo: jax.Array,
    B_x: jax.Array,
    B_k_cache: jax.Array,
    B_v_cache: jax.Array,
    B_wq: jax.Array,
    B_wo: jax.Array,
):
    B, Sq, D = A_x.shape
    _, Hkv, Sk, Dh = A_k_cache.shape
    HD = A_wq.shape[1]
    rep = HD // Dh // Hkv
    scale = (Dh ** -0.5) * LOG2E
    W = rep * Dh
    M = B * Sq
    T = LANES
    EX = Sq - T
    G = T // EX
    U = 2 * Hkv
    NQ = 4
    QW = HD // NQ
    CK = 256
    NC = Sk // CK
    R0, NR = 256, 4
    RC = (M - R0) // NR
    TAIL = 400
    assert 0 < EX and G * Sq == (G + 1) * T and B % G == 0 and EX % 16 == 0
    assert RC * NR + R0 == M and RC % 16 == 0 and R0 % 16 == 0 and QW % W == 0 and (2 * D) % LANES == 0

    def kernel(ax, ak, av, awq, awo, bx, bk, bv, bwq, bwo, out,
               x_s, wq_s, q_s, wo_s, kv_s, out_s, acc_s, zero_s,
               sem_x, sem_wq, sem_wo, sem_kv, sem_out, sem_r, *o_s):
        kv_hbm = (ak, av, bk, bv)
        wq_hbm = (awq, bwq)
        wo_hbm = (awo, bwo)

        def xa0_copy():
            return pltpu.make_async_copy(ax.at[pl.ds(0, R0)], x_s.at[0, pl.ds(0, R0)], sem_r.at[NR])

        def xa_copy(k):
            r = pl.ds(pl.multiple_of(R0 + k * RC, 16), RC)
            return pltpu.make_async_copy(ax.at[r], x_s.at[0, r], sem_r.at[k])

        def xb_copy():
            return pltpu.make_async_copy(bx, x_s.at[1], sem_x.at[0])

        def wq0_copy(k):
            c = pl.ds(k * (QW // 2), QW // 2)
            return pltpu.make_async_copy(awq.at[:, c], wq_s.at[0, :, c], sem_r.at[NR + 1 + k])

        def wq_copy(i):
            return pltpu.make_async_copy(wq_hbm[i // NQ].at[:, pl.ds((i % NQ) * QW, QW)], wq_s.at[i], sem_wq.at[i])

        def wo_copy(blk):
            return pltpu.make_async_copy(wo_hbm[blk], wo_s.at[blk], sem_wo.at[0])

        def kv_copy(i, bb, s):
            return pltpu.make_async_copy(kv_hbm[i].at[bb], kv_s.at[s, i], sem_kv.at[s])

        def out_copy(t):
            r = pl.ds(pl.multiple_of(t * T, T), T)
            return pltpu.make_async_copy(out_s.at[r], out.at[r], sem_out.at[0])

        def q_piece(r, c0, c1):
            q = jnp.dot(x_s[0, r, :], wq_s[0, :, c0:c1], preferred_element_type=F32)
            q_s[0, r, c0:c1] = (q * scale).astype(BF16)

        wq0_copy(0).start()
        xa0_copy().start()
        acc_s[...] = jnp.zeros(acc_s.shape, F32)
        zero_s[0] = 0
        wq0_copy(0).wait()
        wq0_copy(1).start()
        xa_copy(0).start()
        xa0_copy().wait()
        q_piece(pl.ds(0, R0), 0, QW // 2)
        xa_copy(1).start()
        wq0_copy(1).wait()
        q_piece(pl.ds(0, R0), QW // 2, QW)

        def ramp_iter(k, carry):
            xa_copy(k).wait()

            @pl.when(k == 0)
            def _():
                for kk in range(2, NR):
                    xa_copy(kk).start()
                wq_copy(1).start()

            @pl.when(k == 1)
            def _():
                for ii in range(2, 2 * NQ):
                    wq_copy(ii).start()
                xb_copy().start()

            q_piece(pl.ds(pl.multiple_of(R0 + k * RC, 16), RC), 0, QW)
            return carry

        lax.fori_loop(0, NR, ramp_iter, 0)

        def q_iter(i, carry):
            pltpu.make_async_copy(wq_s.at[i], wq_s.at[i], sem_wq.at[i]).wait()

            @pl.when(i == NQ)
            def _():
                xb_copy().wait()

            @pl.when(i == 1)
            def _():
                for blk in range(2):
                    wo_copy(blk).start()
                for ii in range(4):
                    kv_copy(ii, 0, 0).start()

            @pl.when(i == 3)
            def _():
                for ii in range(4):
                    kv_copy(ii, 1, 1).start()

            q = jnp.dot(x_s[i // NQ], wq_s[i], preferred_element_type=F32)
            q_s[i] = (q * scale).astype(BF16)
            return carry

        lax.fori_loop(1, 2 * NQ, q_iter, 0)
        pltpu.make_async_copy(wo_s, wo_s, sem_wo.at[0]).wait()

        def stage(t):
            tt = acc_s[...].T
            out_s[pl.ds(pl.multiple_of(t * T, T), T), :] = tt.astype(BF16)
            z = tt[T - 8:T, 0:LANES]
            for i in range(1, 2 * D // LANES):
                z = z + tt[T - 8:T, i * LANES:(i + 1) * LANES]
            return z

        def o_proj(u, r0, lo=0, hi=D):
            blk, h = u % 2, u // 2
            return lax.dot_general(wo_s[blk, lo:hi, h * W:(h + 1) * W], o_s[u][r0:r0 + T, :], NT,
                                   preferred_element_type=F32)

        def batch_step(g, j):
            b = g * G + j
            slot = lax.bitwise_and(j, 1)
            pltpu.make_async_copy(kv_s.at[slot], kv_s.at[slot], sem_kv.at[slot]).wait()
            zmask = zero_s[0]

            def tie(x):
                return lax.bitcast_convert_type(lax.bitcast_convert_type(x, jnp.int32) & zmask, F32)

            t_prev = jnp.maximum(b - 1 + g, 0)
            staged = stage(t_prev)

            @pl.when(b >= 1)
            def _():
                out_copy(t_prev).start()

            row0 = pl.multiple_of(b * Sq, 16)
            orow = pl.multiple_of(j * EX, 16)

            def scores(u, c):
                blk, h = u % 2, u // 2
                qi, c0 = blk * NQ + (h * W) // QW, (h * W) % QW
                q = jnp.concatenate(
                    [q_s[qi, pl.ds(row0, Sq), c0 + r * Dh:c0 + (r + 1) * Dh] for r in range(rep)], axis=0)
                return lax.dot_general(q, kv_s[slot, 2 * blk, h, c * CK:(c + 1) * CK, :], NT,
                                       preferred_element_type=F32)

            def attend(u, s):
                blk, h = u % 2, u // 2
                m = jnp.max(s, axis=-1, keepdims=True)
                p = jnp.exp2(s - m)
                lp = p[:, 0:LANES]
                for i in range(1, Sk // LANES):
                    lp = lp + p[:, i * LANES:(i + 1) * LANES]
                o = None
                for c in range(NC):
                    a = jnp.dot(p[:, c * CK:(c + 1) * CK].astype(BF16),
                                kv_s[slot, 2 * blk + 1, h, c * CK:(c + 1) * CK, :], preferred_element_type=F32)
                    o = a if o is None else a + o
                lp = lp + tie(o[:, 0:LANES])
                if u == 1:
                    lp = jnp.concatenate([lp[0:8] + tie(staged), lp[8:]], axis=0)
                o = o * (1.0 / jnp.sum(lp, axis=-1, keepdims=True))
                for r in range(rep):
                    o_s[u][pl.ds(orow, Sq), r * Dh:(r + 1) * Dh] = o[r * Sq:(r + 1) * Sq].astype(BF16)

            acc = [None, None]

            def carry_over(u):
                o_s[u][0:T, :] = o_s[u][T:2 * T, :]

            def project(u):
                r = o_proj(u, 0)
                acc[u % 2] = r if acc[u % 2] is None else r + acc[u % 2]
                carry_over(u)

            us, n = U - 2, D - TAIL
            head = None
            for u in range(U):
                ss = []
                for c in range(NC):
                    if c == NC // 2 and u >= 1:
                        if u - 1 == us:
                            head = o_proj(us, 0, 0, n) + acc[us % 2][0:n]
                        else:
                            project(u - 1)
                    ss.append(scores(u, c))
                attend(u, jnp.concatenate(ss, axis=1))
            tail = o_proj(us, 0, n, D) + acc[us % 2][n:D]
            acc[us % 2] = jnp.concatenate([head, tail], axis=0)
            carry_over(us)
            project(U - 1)
            acc_s[0:D, :] = acc[0]
            acc_s[D:2 * D, :] = acc[1]

            @pl.when(b + 2 < B)
            def _():
                for i in range(4):
                    kv_copy(i, b + 2, slot).start()

        def group(g, carry):
            def body(j, c2):
                batch_step(g, j)
                return c2

            lax.fori_loop(0, G, body, 0)
            t_last = g * (G + 1) + G - 1
            stage(t_last)
            out_copy(t_last).start()
            acc = [None, None]
            for u in range(U):
                r = o_proj(u, T)
                acc[u % 2] = r if acc[u % 2] is None else r + acc[u % 2]
            acc_s[0:D, :] = acc[0]
            acc_s[D:2 * D, :] = acc[1]
            return carry

        lax.fori_loop(0, B // G, group, 0)
        stage(M // T - 1)
        out_copy(M // T - 1).start()
        pltpu.make_async_copy(out_s, out, sem_out.at[0]).wait()

    any_spec = pl.BlockSpec(memory_space=pl.ANY)
    out = pl.pallas_call(
        kernel,
        in_specs=[any_spec] * 10,
        out_specs=any_spec,
        out_shape=jax.ShapeDtypeStruct((M, 2 * D), BF16),
        scratch_shapes=[
            pltpu.VMEM((2, M, D), BF16),
            pltpu.VMEM((2 * NQ, D, QW), BF16),
            pltpu.VMEM((2 * NQ, M, QW), BF16),
            pltpu.VMEM((2, D, HD), BF16),
            pltpu.VMEM((2, 4, Hkv, Sk, Dh), BF16),
            pltpu.VMEM((M, 2 * D), BF16),
            pltpu.VMEM((2 * D, T), F32),
            pltpu.SMEM((1,), jnp.int32),
            pltpu.SemaphoreType.DMA((1,)),
            pltpu.SemaphoreType.DMA((2 * NQ,)),
            pltpu.SemaphoreType.DMA((1,)),
            pltpu.SemaphoreType.DMA((2,)),
            pltpu.SemaphoreType.DMA((1,)),
            pltpu.SemaphoreType.DMA((NR + 3,)),
        ] + [pltpu.VMEM((2 * T, W), BF16)] * U,
        compiler_params=pltpu.CompilerParams(
            vmem_limit_bytes=120 * 1024 * 1024,
            disable_bounds_checks=True),
    )(A_x.reshape(M, D), A_k_cache, A_v_cache, A_wq, A_wo.T,
      B_x.reshape(M, D), B_k_cache, B_v_cache, B_wq, B_wo.T)
    return out.reshape(B, Sq, 2 * D)
```

```python
import jax
import jax.numpy as jnp
from jax import lax
import jax.experimental.pallas as pl
import jax.experimental.pallas.tpu as pltpu

LOG2E = 1.4426950408889634
NT = (((1,), (1,)), ((), ()))
BF16 = jnp.bfloat16
F32 = jnp.float32
LANES = 128


@jax.jit
def pallas_concat_heads__gqa_block_cached__gqa_block_cached__near_ridge_kernel(
    A_x: jax.Array,
    A_k_cache: jax.Array,
    A_v_cache: jax.Array,
    A_wq: jax.Array,
    A_wo: jax.Array,
    B_x: jax.Array,
    B_k_cache: jax.Array,
    B_v_cache: jax.Array,
    B_wq: jax.Array,
    B_wo: jax.Array,
):
    B, Sq, D = A_x.shape
    _, Hkv, Sk, Dh = A_k_cache.shape
    HD = A_wq.shape[1]
    rep = HD // Dh // Hkv
    scale = (Dh ** -0.5) * LOG2E
    W = rep * Dh
    M = B * Sq
    T = LANES
    EX = Sq - T
    G = T // EX
    U = 2 * Hkv
    NQ = 4
    QW = HD // NQ
    CK = 256
    NC = Sk // CK
    R0, NR = 256, 4
    RC = (M - R0) // NR
    TAIL = 400
    assert 0 < EX and G * Sq == (G + 1) * T and B % G == 0 and EX % 16 == 0
    assert RC * NR + R0 == M and RC % 16 == 0 and R0 % 16 == 0 and QW % W == 0 and (2 * D) % LANES == 0

    def kernel(ax, ak, av, awq, awo, bx, bk, bv, bwq, bwo, out,
               x_s, wq_s, q_s, wo_s, kv_s, out_s, acc_s, zero_s,
               sem_x, sem_wq, sem_wo, sem_kv, sem_out, sem_r, *o_s):
        kv_hbm = (ak, av, bk, bv)
        wq_hbm = (awq, bwq)
        wo_hbm = (awo, bwo)

        def xa0_copy():
            return pltpu.make_async_copy(ax.at[pl.ds(0, R0)], x_s.at[0, pl.ds(0, R0)], sem_r.at[NR])

        def xa_copy(k):
            r = pl.ds(pl.multiple_of(R0 + k * RC, 16), RC)
            return pltpu.make_async_copy(ax.at[r], x_s.at[0, r], sem_r.at[k])

        def xb_copy():
            return pltpu.make_async_copy(bx, x_s.at[1], sem_x.at[0])

        def wq0_copy(k):
            c = pl.ds(k * (QW // 2), QW // 2)
            return pltpu.make_async_copy(awq.at[:, c], wq_s.at[0, :, c], sem_r.at[NR + 1 + k])

        def wq_copy(i):
            return pltpu.make_async_copy(wq_hbm[i // NQ].at[:, pl.ds((i % NQ) * QW, QW)], wq_s.at[i], sem_wq.at[i])

        def wo_copy(blk):
            return pltpu.make_async_copy(wo_hbm[blk], wo_s.at[blk], sem_wo.at[0])

        def kv_copy(i, bb, s):
            return pltpu.make_async_copy(kv_hbm[i].at[bb], kv_s.at[s, i], sem_kv.at[s])

        def out_copy(t):
            r = pl.ds(pl.multiple_of(t * T, T), T)
            return pltpu.make_async_copy(out_s.at[r], out.at[r], sem_out.at[0])

        def q_piece(r, c0, c1):
            q = jnp.dot(x_s[0, r, :], wq_s[0, :, c0:c1], preferred_element_type=F32)
            q_s[0, r, c0:c1] = (q * scale).astype(BF16)

        g = pl.program_id(0)

        @pl.when(g == 0)
        def _():
            wq0_copy(0).start()
            xa0_copy().start()
            acc_s[...] = jnp.zeros(acc_s.shape, F32)
            zero_s[0] = 0
            wq0_copy(0).wait()
            wq0_copy(1).start()
            xa_copy(0).start()
            xa0_copy().wait()
            q_piece(pl.ds(0, R0), 0, QW // 2)
            xa_copy(1).start()
            wq0_copy(1).wait()
            q_piece(pl.ds(0, R0), QW // 2, QW)

            def ramp_iter(k, carry):
                xa_copy(k).wait()

                @pl.when(k == 0)
                def _():
                    for kk in range(2, NR):
                        xa_copy(kk).start()
                    wq_copy(1).start()

                @pl.when(k == 1)
                def _():
                    for ii in range(2, 2 * NQ):
                        wq_copy(ii).start()
                    xb_copy().start()

                q_piece(pl.ds(pl.multiple_of(R0 + k * RC, 16), RC), 0, QW)
                return carry

            lax.fori_loop(0, NR, ramp_iter, 0)

            def q_iter(i, carry):
                pltpu.make_async_copy(wq_s.at[i], wq_s.at[i], sem_wq.at[i]).wait()

                @pl.when(i == NQ)
                def _():
                    xb_copy().wait()

                @pl.when(i == 1)
                def _():
                    for blk in range(2):
                        wo_copy(blk).start()
                    for ii in range(4):
                        kv_copy(ii, 0, 0).start()

                @pl.when(i == 3)
                def _():
                    for ii in range(4):
                        kv_copy(ii, 1, 1).start()

                q = jnp.dot(x_s[i // NQ], wq_s[i], preferred_element_type=F32)
                q_s[i] = (q * scale).astype(BF16)
                return carry

            lax.fori_loop(1, 2 * NQ, q_iter, 0)
            pltpu.make_async_copy(wo_s, wo_s, sem_wo.at[0]).wait()

        def stage(t):
            tt = acc_s[...].T
            out_s[pl.ds(pl.multiple_of(t * T, T), T), :] = tt.astype(BF16)
            z = tt[T - 8:T, 0:LANES]
            for i in range(1, 2 * D // LANES):
                z = z + tt[T - 8:T, i * LANES:(i + 1) * LANES]
            return z

        def o_proj(u, r0, lo=0, hi=D):
            blk, h = u % 2, u // 2
            return lax.dot_general(wo_s[blk, lo:hi, h * W:(h + 1) * W], o_s[u][r0:r0 + T, :], NT,
                                   preferred_element_type=F32)

        def batch_step(g, j):
            b = g * G + j
            slot = lax.bitwise_and(j, 1)
            pltpu.make_async_copy(kv_s.at[slot], kv_s.at[slot], sem_kv.at[slot]).wait()
            zmask = zero_s[0]

            def tie(x):
                return lax.bitcast_convert_type(lax.bitcast_convert_type(x, jnp.int32) & zmask, F32)

            t_prev = jnp.maximum(b - 1 + g, 0)
            staged = stage(t_prev)

            @pl.when(b >= 1)
            def _():
                out_copy(t_prev).start()

            row0 = pl.multiple_of(b * Sq, 16)
            orow = pl.multiple_of(j * EX, 16)

            def scores(u, c):
                blk, h = u % 2, u // 2
                qi, c0 = blk * NQ + (h * W) // QW, (h * W) % QW
                q = jnp.concatenate(
                    [q_s[qi, pl.ds(row0, Sq), c0 + r * Dh:c0 + (r + 1) * Dh] for r in range(rep)], axis=0)
                return lax.dot_general(q, kv_s[slot, 2 * blk, h, c * CK:(c + 1) * CK, :], NT,
                                       preferred_element_type=F32)

            def attend(u, s):
                blk, h = u % 2, u // 2
                m = jnp.max(s, axis=-1, keepdims=True)
                p = jnp.exp2(s - m)
                lp = p[:, 0:LANES]
                for i in range(1, Sk // LANES):
                    lp = lp + p[:, i * LANES:(i + 1) * LANES]
                o = None
                for c in range(NC):
                    a = jnp.dot(p[:, c * CK:(c + 1) * CK].astype(BF16),
                                kv_s[slot, 2 * blk + 1, h, c * CK:(c + 1) * CK, :], preferred_element_type=F32)
                    o = a if o is None else a + o
                lp = lp + tie(o[:, 0:LANES])
                if u == 1:
                    lp = jnp.concatenate([lp[0:8] + tie(staged), lp[8:]], axis=0)
                o = o * (1.0 / jnp.sum(lp, axis=-1, keepdims=True))
                for r in range(rep):
                    o_s[u][pl.ds(orow, Sq), r * Dh:(r + 1) * Dh] = o[r * Sq:(r + 1) * Sq].astype(BF16)

            acc = [None, None]

            def carry_over(u):
                o_s[u][0:T, :] = o_s[u][T:2 * T, :]

            def project(u):
                r = o_proj(u, 0)
                acc[u % 2] = r if acc[u % 2] is None else r + acc[u % 2]
                carry_over(u)

            us, n = U - 2, D - TAIL
            head = None
            for u in range(U):
                ss = []
                for c in range(NC):
                    if c == NC // 2 and u >= 1:
                        if u - 1 == us:
                            head = o_proj(us, 0, 0, n) + acc[us % 2][0:n]
                        else:
                            project(u - 1)
                    ss.append(scores(u, c))
                attend(u, jnp.concatenate(ss, axis=1))
            tail = o_proj(us, 0, n, D) + acc[us % 2][n:D]
            acc[us % 2] = jnp.concatenate([head, tail], axis=0)
            carry_over(us)
            project(U - 1)
            acc_s[0:D, :] = acc[0]
            acc_s[D:2 * D, :] = acc[1]

            @pl.when(b + 2 < B)
            def _():
                for i in range(4):
                    kv_copy(i, b + 2, slot).start()

        def body(j, c2):
            batch_step(g, j)
            return c2

        lax.fori_loop(0, G, body, 0)
        t_last = g * (G + 1) + G - 1
        stage(t_last)
        out_copy(t_last).start()
        acc = [None, None]
        for u in range(U):
            r = o_proj(u, T)
            acc[u % 2] = r if acc[u % 2] is None else r + acc[u % 2]
        acc_s[0:D, :] = acc[0]
        acc_s[D:2 * D, :] = acc[1]

        @pl.when(g == B // G - 1)
        def _():
            stage(M // T - 1)
            out_copy(M // T - 1).start()
            pltpu.make_async_copy(out_s, out, sem_out.at[0]).wait()

    any_spec = pl.BlockSpec(memory_space=pl.ANY)
    out = pl.pallas_call(
        kernel,
        grid=(B // G,),
        in_specs=[any_spec] * 10,
        out_specs=any_spec,
        out_shape=jax.ShapeDtypeStruct((M, 2 * D), BF16),
        scratch_shapes=[
            pltpu.VMEM((2, M, D), BF16),
            pltpu.VMEM((2 * NQ, D, QW), BF16),
            pltpu.VMEM((2 * NQ, M, QW), BF16),
            pltpu.VMEM((2, D, HD), BF16),
            pltpu.VMEM((2, 4, Hkv, Sk, Dh), BF16),
            pltpu.VMEM((M, 2 * D), BF16),
            pltpu.VMEM((2 * D, T), F32),
            pltpu.SMEM((1,), jnp.int32),
            pltpu.SemaphoreType.DMA((1,)),
            pltpu.SemaphoreType.DMA((2 * NQ,)),
            pltpu.SemaphoreType.DMA((1,)),
            pltpu.SemaphoreType.DMA((2,)),
            pltpu.SemaphoreType.DMA((1,)),
            pltpu.SemaphoreType.DMA((NR + 3,)),
        ] + [pltpu.VMEM((2 * T, W), BF16)] * U,
        compiler_params=pltpu.CompilerParams(
            dimension_semantics=("arbitrary",),
            vmem_limit_bytes=120 * 1024 * 1024,
            disable_bounds_checks=True,
            disable_semaphore_checks=True),
    )(A_x.reshape(M, D), A_k_cache, A_v_cache, A_wq, A_wo.T,
      B_x.reshape(M, D), B_k_cache, B_v_cache, B_wq, B_wo.T)
    return out.reshape(B, Sq, 2 * D)
```

```python
import jax
import jax.numpy as jnp
from jax import lax
import jax.experimental.pallas as pl
import jax.experimental.pallas.tpu as pltpu

LOG2E = 1.4426950408889634
NT = (((1,), (1,)), ((), ()))
BF16 = jnp.bfloat16
F32 = jnp.float32
LANES = 128


@jax.jit
def pallas_concat_heads__gqa_block_cached__gqa_block_cached__near_ridge_kernel(
    A_x: jax.Array,
    A_k_cache: jax.Array,
    A_v_cache: jax.Array,
    A_wq: jax.Array,
    A_wo: jax.Array,
    B_x: jax.Array,
    B_k_cache: jax.Array,
    B_v_cache: jax.Array,
    B_wq: jax.Array,
    B_wo: jax.Array,
):
    B, Sq, D = A_x.shape
    _, Hkv, Sk, Dh = A_k_cache.shape
    HD = A_wq.shape[1]
    rep = HD // Dh // Hkv
    scale = (Dh ** -0.5) * LOG2E
    W = rep * Dh
    M = B * Sq
    T = LANES
    EX = Sq - T
    G = T // EX
    U = 2 * Hkv
    NQ = 4
    QW = HD // NQ
    CK = 256
    NC = Sk // CK
    R0, NR = 256, 4
    RC = (M - R0) // NR
    TAIL = 400
    assert 0 < EX and G * Sq == (G + 1) * T and B % G == 0 and G % 2 == 0 and EX % 16 == 0
    assert RC * NR + R0 == M and RC % 16 == 0 and R0 % 16 == 0 and QW % W == 0 and (2 * D) % LANES == 0

    def kernel(ax, ak, av, awq, awo, bx, bk, bv, bwq, bwo, out,
               x_s, wq_s, q_s, wo_s, kv_s, out_s, acc_s, zero_s,
               sem_x, sem_wq, sem_wo, sem_kv, sem_out, sem_r, *o_s):
        kv_hbm = (ak, av, bk, bv)
        wq_hbm = (awq, bwq)
        wo_hbm = (awo, bwo)

        def xa0_copy():
            return pltpu.make_async_copy(ax.at[pl.ds(0, R0)], x_s.at[0, pl.ds(0, R0)], sem_r.at[NR])

        def xa_copy(k):
            r = pl.ds(pl.multiple_of(R0 + k * RC, 16), RC)
            return pltpu.make_async_copy(ax.at[r], x_s.at[0, r], sem_r.at[k])

        def xb_copy():
            return pltpu.make_async_copy(bx, x_s.at[1], sem_x.at[0])

        def wq0_copy(k):
            c = pl.ds(k * (QW // 2), QW // 2)
            return pltpu.make_async_copy(awq.at[:, c], wq_s.at[0, :, c], sem_r.at[NR + 1 + k])

        def wq_copy(i):
            return pltpu.make_async_copy(wq_hbm[i // NQ].at[:, pl.ds((i % NQ) * QW, QW)], wq_s.at[i], sem_wq.at[i])

        def wo_copy(blk):
            return pltpu.make_async_copy(wo_hbm[blk], wo_s.at[blk], sem_wo.at[0])

        def kv_copy(i, bb, s):
            return pltpu.make_async_copy(kv_hbm[i].at[bb], kv_s.at[s, i], sem_kv.at[s])

        def out_copy(t):
            r = pl.ds(pl.multiple_of(t * T, T), T)
            return pltpu.make_async_copy(out_s.at[r], out.at[r], sem_out.at[0])

        def q_piece(r, c0, c1):
            q = jnp.dot(x_s[0, r, :], wq_s[0, :, c0:c1], preferred_element_type=F32)
            q_s[0, r, c0:c1] = (q * scale).astype(BF16)

        g = pl.program_id(0)

        @pl.when(g == 0)
        def _():
            wq0_copy(0).start()
            xa0_copy().start()
            acc_s[...] = jnp.zeros(acc_s.shape, F32)
            zero_s[0] = 0

            def clear(k, carry):
                for u in range(U):
                    o_s[u][pl.ds(pl.multiple_of(k * 32, 32), 32), :] = jnp.zeros((32, W), BF16)
                return carry

            lax.fori_loop(0, 2 * T // 32, clear, 0)
            wq0_copy(0).wait()
            wq0_copy(1).start()
            xa_copy(0).start()
            xa0_copy().wait()
            q_piece(pl.ds(0, R0), 0, QW // 2)
            xa_copy(1).start()
            wq0_copy(1).wait()
            q_piece(pl.ds(0, R0), QW // 2, QW)

            def ramp_iter(k, carry):
                xa_copy(k).wait()

                @pl.when(k == 0)
                def _():
                    for kk in range(2, NR):
                        xa_copy(kk).start()
                    wq_copy(1).start()

                @pl.when(k == 1)
                def _():
                    for ii in range(2, 2 * NQ):
                        wq_copy(ii).start()
                    xb_copy().start()

                q_piece(pl.ds(pl.multiple_of(R0 + k * RC, 16), RC), 0, QW)
                return carry

            lax.fori_loop(0, NR, ramp_iter, 0)

            def q_iter(i, carry):
                pltpu.make_async_copy(wq_s.at[i], wq_s.at[i], sem_wq.at[i]).wait()

                @pl.when(i == NQ)
                def _():
                    xb_copy().wait()

                @pl.when(i == 1)
                def _():
                    for blk in range(2):
                        wo_copy(blk).start()
                    for ii in range(4):
                        kv_copy(ii, 0, 0).start()

                @pl.when(i == 3)
                def _():
                    for ii in range(4):
                        kv_copy(ii, 1, 1).start()

                q = jnp.dot(x_s[i // NQ], wq_s[i], preferred_element_type=F32)
                q_s[i] = (q * scale).astype(BF16)
                return carry

            lax.fori_loop(1, 2 * NQ, q_iter, 0)
            pltpu.make_async_copy(wo_s, wo_s, sem_wo.at[0]).wait()

        def stage(t):
            tt = acc_s[...].T
            out_s[pl.ds(pl.multiple_of(t * T, T), T), :] = tt.astype(BF16)
            z = tt[T - 8:T, 0:LANES]
            for i in range(1, 2 * D // LANES):
                z = z + tt[T - 8:T, i * LANES:(i + 1) * LANES]
            return z

        def o_proj(u, r0, lo=0, hi=D):
            blk, h = u % 2, u // 2
            return lax.dot_general(wo_s[blk, lo:hi, h * W:(h + 1) * W], o_s[u][r0:r0 + T, :], NT,
                                   preferred_element_type=F32)

        def batch_step(g, j):
            b = g * G + j
            slot = lax.bitwise_and(j, 1)
            pltpu.make_async_copy(kv_s.at[slot], kv_s.at[slot], sem_kv.at[slot]).wait()
            zmask = zero_s[0]

            def tie(x):
                return lax.bitcast_convert_type(lax.bitcast_convert_type(x, jnp.int32) & zmask, F32)

            t_prev = jnp.maximum(b - 1 + g, 0)
            staged = stage(t_prev)

            @pl.when(b >= 1)
            def _():
                out_copy(t_prev).start()

            row0 = pl.multiple_of(b * Sq, 16)
            orow = pl.multiple_of(j * EX, 16)

            def scores(u, c):
                blk, h = u % 2, u // 2
                qi, c0 = blk * NQ + (h * W) // QW, (h * W) % QW
                q = jnp.concatenate(
                    [q_s[qi, pl.ds(row0, Sq), c0 + r * Dh:c0 + (r + 1) * Dh] for r in range(rep)], axis=0)
                return lax.dot_general(q, kv_s[slot, 2 * blk, h, c * CK:(c + 1) * CK, :], NT,
                                       preferred_element_type=F32)

            def attend(u, s):
                blk, h = u % 2, u // 2
                m = jnp.max(s, axis=-1, keepdims=True)
                p = jnp.exp2(s - m)
                lp = p[:, 0:LANES]
                for i in range(1, Sk // LANES):
                    lp = lp + p[:, i * LANES:(i + 1) * LANES]
                o = None
                for c in range(NC):
                    a = jnp.dot(p[:, c * CK:(c + 1) * CK].astype(BF16),
                                kv_s[slot, 2 * blk + 1, h, c * CK:(c + 1) * CK, :], preferred_element_type=F32)
                    o = a if o is None else a + o
                lp = lp + tie(o[:, 0:LANES])
                if u == 1:
                    lp = jnp.concatenate([lp[0:8] + tie(staged), lp[8:]], axis=0)
                o = o * (1.0 / jnp.sum(lp, axis=-1, keepdims=True))
                for r in range(rep):
                    o_s[u][pl.ds(orow, Sq), r * Dh:(r + 1) * Dh] = o[r * Sq:(r + 1) * Sq].astype(BF16)

            acc = [None, None]

            def carry_over(u):
                o_s[u][0:T, :] = o_s[u][T:2 * T, :]

            def project(u):
                r = o_proj(u, 0)
                acc[u % 2] = r if acc[u % 2] is None else r + acc[u % 2]
                carry_over(u)

            us, n = U - 2, D - TAIL
            head = None
            for u in range(U):
                ss = []
                for c in range(NC):
                    if c == NC // 2 and u >= 1:
                        if u - 1 == us:
                            head = o_proj(us, 0, 0, n) + acc[us % 2][0:n]
                        else:
                            project(u - 1)
                    ss.append(scores(u, c))
                attend(u, jnp.concatenate(ss, axis=1))
            tail = o_proj(us, 0, n, D) + acc[us % 2][n:D]
            acc[us % 2] = jnp.concatenate([head, tail], axis=0)
            carry_over(us)
            project(U - 1)
            acc_s[0:D, :] = acc[0]
            acc_s[D:2 * D, :] = acc[1]

            @pl.when(b + 2 < B)
            def _():
                for i in range(4):
                    kv_copy(i, b + 2, slot).start()

        def body(j, c2):
            batch_step(g, j)
            return c2

        lax.fori_loop(0, G, body, 0)
        t_last = g * (G + 1) + G - 1
        stage(t_last)
        out_copy(t_last).start()
        acc = [None, None]
        for u in range(U):
            r = o_proj(u, T)
            acc[u % 2] = r if acc[u % 2] is None else r + acc[u % 2]
        acc_s[0:D, :] = acc[0]
        acc_s[D:2 * D, :] = acc[1]

        @pl.when(g == B // G - 1)
        def _():
            stage(M // T - 1)
            out_copy(M // T - 1).start()
            pltpu.make_async_copy(out_s, out, sem_out.at[0]).wait()

    any_spec = pl.BlockSpec(memory_space=pl.ANY)
    out = pl.pallas_call(
        kernel,
        grid=(B // G,),
        in_specs=[any_spec] * 10,
        out_specs=any_spec,
        out_shape=jax.ShapeDtypeStruct((M, 2 * D), BF16),
        scratch_shapes=[
            pltpu.VMEM((2, M, D), BF16),
            pltpu.VMEM((2 * NQ, D, QW), BF16),
            pltpu.VMEM((2 * NQ, M, QW), BF16),
            pltpu.VMEM((2, D, HD), BF16),
            pltpu.VMEM((2, 4, Hkv, Sk, Dh), BF16),
            pltpu.VMEM((M, 2 * D), BF16),
            pltpu.VMEM((2 * D, T), F32),
            pltpu.SMEM((1,), jnp.int32),
            pltpu.SemaphoreType.DMA((1,)),
            pltpu.SemaphoreType.DMA((2 * NQ,)),
            pltpu.SemaphoreType.DMA((1,)),
            pltpu.SemaphoreType.DMA((2,)),
            pltpu.SemaphoreType.DMA((1,)),
            pltpu.SemaphoreType.DMA((NR + 3,)),
        ] + [pltpu.VMEM((2 * T, W), BF16)] * U,
        compiler_params=pltpu.CompilerParams(
            dimension_semantics=("arbitrary",),
            vmem_limit_bytes=120 * 1024 * 1024,
            disable_bounds_checks=True,
            disable_semaphore_checks=True),
    )(A_x.reshape(M, D), A_k_cache, A_v_cache, A_wq, A_wo.T,
      B_x.reshape(M, D), B_k_cache, B_v_cache, B_wq, B_wo.T)
    return out.reshape(B, Sq, 2 * D)
```
